```python
import os as _os
_os.environ.setdefault("JAX_PLATFORMS", "cpu")
import jax
import jax.numpy as jnp

def _softmax(x, axis=-1):
    return jax.nn.softmax(x, axis=axis)
def _gelu(x):
    return jax.nn.gelu(x, approximate=True)
def _silu(x):
    return jax.nn.silu(x)
def _sigmoid(x):
    return jax.nn.sigmoid(x)
def _layernorm(x, axis=-1, eps=1e-5):
    m = jnp.mean(x, axis=axis, keepdims=True)
    v = jnp.var(x, axis=axis, keepdims=True)
    return (x - m) / jnp.sqrt(v + eps)
def _scatter_add(tgt, idx, src, axis=0):
    return tgt.at[idx].add(src)
def _segment_sum(src, seg, n):
    return jax.ops.segment_sum(src, seg, n)
class _Rng:
    def __init__(self, key):
        self._k = key
    def _next(self):
        self._k, sub = jax.random.split(self._k)
        return sub
    def normal(self, shape):
        return jax.random.normal(self._next(), shape, dtype=jnp.bfloat16)
    def randint(self, lo, hi, shape):
        return jax.random.randint(self._next(), shape, lo, hi, dtype=jnp.int32)
    def uniform(self, shape, lo=0.0, hi=1.0):
        return jax.random.uniform(self._next(), shape, jnp.bfloat16, lo, hi)
    def permutation(self, n):
        return jax.random.permutation(self._next(), n)


kernel_name = 'standalone__layernorm_linear__sampling'

def setup_inputs():
    _rng = _Rng(jax.random.key(int.from_bytes(__import__("os").urandom(4), "little")))
    _w = (lambda a: (lambda t: t.astype(jnp.bfloat16) if jnp.issubdtype(t.dtype, jnp.floating) else t)(jnp.asarray(a)))
    B, S, D = 1024, 32, 576
    return {
        "x": _w((lambda *s: _rng.normal(s) * 0.05)(B, S, D)),
        "g": _w((lambda *s: _rng.normal(s) * 0.05)(D) + 1.0),
        "b": _w((lambda *s: _rng.normal(s) * 0.05)(D)),
        "w": _w((lambda *s: _rng.normal(s) * 0.05)(D, D)),
    }

def reference(x, g, b, w):
    return (_layernorm(x, axis=-1) * g + b) @ w
```

```python
import jax
import jax.numpy as jnp
from jax import lax
import jax.experimental.pallas as pl
import jax.experimental.pallas.tpu as pltpu

D = 576
H = D // 2
NS = 32
EPS = 1e-5
WSTART = 15
f32, bf16, u32 = jnp.float32, jnp.bfloat16, jnp.uint32


def _pk(v):
    return pltpu.bitcast(v.astype(bf16), u32)


def _up(v):
    return pltpu.bitcast(v, bf16)


def _kernel(x_hbm, g_ref, b_ref, w_ref, o_hbm, xbuf, obuf, at, ar, bias_ref, rsem, wsem):
    def rd(s):
        return pltpu.make_async_copy(x_hbm.at[s], xbuf.at[s], rsem.at[s])

    def wr(s):
        return pltpu.make_async_copy(obuf.at[s], o_hbm.at[s], wsem.at[s])

    for s in range(NS):
        rd(s).start()
    g = g_ref[...].astype(f32)
    b = b_ref[...].astype(f32)
    wt = w_ref[...].astype(f32).T
    bias_ref[...] = jnp.broadcast_to(jnp.sum(wt * b, axis=1, keepdims=True), bias_ref.shape)
    wg = wt * g
    t = [wg[:, k * 128:(k + 1) * 128] for k in range(4)]
    t3q = jnp.concatenate([wg[:, 384:448], wg[:, 512:]], axis=1)
    ar[...] = _pk(wg[:, 448:])
    for j, (a1, a2) in enumerate([(t[0], t[2]), (t[1], t[3]), (t[1], t3q)]):
        a11, a21, a12, a22 = a1[:H], a1[H:], a2[:H], a2[H:]
        for m, v in enumerate([a11 + a22, a21 + a22, a11, a22, a11 + a12, a21 - a11, a12 - a22]):
            at[m, j] = _pk(v)

    def ldx(s, p, r0=0, r1=D):
        return xbuf[s, r0:r1, p * 256:(p + 1) * 256].astype(f32)

    def stats(s, p):
        x = ldx(s, p)
        c = x[0:1]
        xc = x - c
        d = jnp.sum(xc, axis=0, keepdims=True) * (1.0 / D)
        var = jnp.sum(xc * xc, axis=0, keepdims=True) * (1.0 / D) - d * d
        return c + d, lax.rsqrt(jnp.maximum(var, 0.0) + EPS)

    def norm(s, p, st, r0, r1):
        return (ldx(s, p, r0, r1) - st[0]) * st[1]

    def rhs_r(s, p, st):
        y = norm(s, p, st, 448, 576)
        return jnp.concatenate([y[:64, 128:], y[64:, :128]], axis=0)

    def half(s, p, st, k):
        if k == 0:
            return norm(s, p, st, 0, 256)
        y = norm(s, p, st, 256, 576)
        tail = jnp.concatenate(
            [y[192:256, :128] - y[192:256, 128:], y[256:, 128:] - y[256:, :128]], axis=1)
        return jnp.concatenate([y[:192], tail], axis=0)

    def prod(m, rhs):
        a0 = _up(at[m, 0])
        mp = jnp.dot(jnp.concatenate([a0, _up(at[m, 1])], axis=1), rhs[:, :128].astype(bf16),
                     preferred_element_type=f32)
        mq = jnp.dot(jnp.concatenate([a0, _up(at[m, 2])], axis=1), rhs[:, 128:].astype(bf16),
                     preferred_element_type=f32)
        return jnp.concatenate([mp, mq], axis=1)

    def quad(s, q, st, rr):
        p0, p1 = 2 * q, 2 * q + 1
        b11, b12 = half(s, p0, st[p0], 0), half(s, p1, st[p1], 0)
        b21, b22 = half(s, p0, st[p0], 1), half(s, p1, st[p1], 1)

        def put(i, p, v):
            r = rr[p][i * H:(i + 1) * H]
            obuf[s, i * H:(i + 1) * H, p * 256:(p + 1) * 256] = (
                v + jnp.concatenate([r, r], axis=1)).astype(bf16)

        m1 = prod(0, b11 + b22)
        m2 = prod(1, b11)
        m3 = prod(2, b12 - b22)
        m4 = prod(3, b21 - b11)
        put(1, p0, m2 + m4)
        m5 = prod(4, b22)
        put(0, p1, m3 + m5)
        m6 = prod(5, b11 + b12)
        put(1, p1, (m3 - m2) + m1 + m6)
        m7 = prod(6, b21 + b22)
        put(0, p0, (m4 - m5) + m1 + m7)

    rd(0).wait()
    st0 = [stats(0, p) for p in range(4)]

    def body(s, st):
        @pl.when(s < NS - 1)
        def _():
            rd(s + 1).wait()

        sn = jnp.minimum(s + 1, NS - 1)
        r = jnp.dot(_up(ar[...]),
                    jnp.concatenate([rhs_r(s, p, st[p]) for p in range(4)], axis=1).astype(bf16),
                    preferred_element_type=f32)
        rr = [r[:, p * 128:(p + 1) * 128] + bias_ref[...] for p in range(4)]
        nst = []
        for q in range(2):
            quad(s, q, st, rr)
            nst += [stats(sn, 2 * q), stats(sn, 2 * q + 1)]

        @pl.when(s == WSTART - 1)
        def _():
            for k in range(WSTART - 1):
                wr(k).start()

        @pl.when(s >= WSTART - 1)
        def _():
            wr(s).start()

        return nst

    lax.fori_loop(0, NS, body, st0)
    for s in range(NS):
        wr(s).wait()


@jax.jit
def pallas_standalone__layernorm_linear__sampling_kernel(
    x: jax.Array,
    g: jax.Array,
    b: jax.Array,
    w: jax.Array,
):
    xt = jnp.transpose(x, (1, 2, 0))
    vmem = pl.BlockSpec(memory_space=pltpu.VMEM)
    o = pl.pallas_call(
        _kernel,
        in_specs=[pl.BlockSpec(memory_space=pl.ANY), vmem, vmem, vmem],
        out_specs=pl.BlockSpec(memory_space=pl.ANY),
        out_shape=jax.ShapeDtypeStruct(xt.shape, xt.dtype),
        scratch_shapes=[
            pltpu.VMEM(xt.shape, bf16), pltpu.VMEM(xt.shape, bf16),
            pltpu.VMEM((7, 3, H // 2, 128), u32), pltpu.VMEM((D // 2, 128), u32),
            pltpu.VMEM((D, 128), f32),
            pltpu.SemaphoreType.DMA((NS,)), pltpu.SemaphoreType.DMA((NS,)),
        ],
        compiler_params=pltpu.CompilerParams(vmem_limit_bytes=100 * 2**20),
    )(xt, g.reshape(1, D), b.reshape(1, D), w)
    return jnp.transpose(o, (2, 0, 1))
```

```python
import functools
import jax, jax.numpy as jnp, numpy as np
from jax import lax
from jax.experimental import pallas as pl
from jax.experimental.pallas import tpu as pltpu

D = 576
H = 288
EPS = 1e-5
NS = 32
f32, bf16, u32 = jnp.float32, jnp.bfloat16, jnp.uint32
OUTS = {(0, 1): {3: 1, 5: 1}, (1, 0): {2: 1, 4: 1}, (0, 0): {1: 1, 4: 1, 5: -1, 7: 1}, (1, 1): {1: 1, 2: -1, 3: 1, 6: 1}}
def acomb(m, a11, a12, a21, a22):
    return {1: lambda: a11 + a22, 2: lambda: a21 + a22, 3: lambda: a11, 4: lambda: a22, 5: lambda: a11 + a12, 6: lambda: a21 - a11, 7: lambda: a12 - a22}[m]()
def bcomb(m, B):
    return {1: lambda: B(0, 0) + B(1, 1), 2: lambda: B(0, 0), 3: lambda: B(0, 1) - B(1, 1), 4: lambda: B(1, 0) - B(0, 0),
            5: lambda: B(1, 1), 6: lambda: B(0, 0) + B(0, 1), 7: lambda: B(1, 0) + B(1, 1)}[m]()
def chain(terms):
    sg, acc = terms[0]
    for sgn, v in terms[1:]:
        if sg > 0: acc = acc + v if sgn > 0 else acc - v
        elif sgn > 0: acc, sg = v - acc, 1
        else: acc = acc + v
    assert sg > 0
    return acc

def make(wstart=15, dma=True, flags=None, sched="2a 6a 3a r 5a 1a 4a 7a 2b 6b 3b 5b 1b 4b 7b", unroll=1, peel=0, nch=12, d0=1.0, d1=13.0,
         nobc=True, wn=12, wgroup=2, nsingle=1, fine=True, groups=None, wstep=0, pwstep=4, pd0=3.0, o2="2635147", split0=2):
    steps = sched.split()
    two = sorted(int(t[0]) for t in steps if t.endswith("x"))
    wr_rows = H // wn
    def pk(v): return pltpu.bitcast(v.astype(bf16), u32)
    def up(v): return pltpu.bitcast(v, bf16)
    last = NS - 1 if fine else NS
    if groups is None:
        groups = [(0, wstart)]
        s = wstart
        while s < last:
            k = wgroup if s + wgroup <= last - nsingle else 1
            groups.append((s, s + k)); s += k
    else: groups = list(zip((0,) + groups[:-1], groups))
    def kern(x_hbm, g_hbm, b_hbm, w_hbm, o_hbm, xbuf, obuf, g_ref, b_ref, w_ref, at, a2, ar, bias_ref, rsem, psem, wsem):
        c0 = 1024 // split0
        def rd(s): return pltpu.make_async_copy(x_hbm.at[s], xbuf.at[s], rsem.at[s])
        def rd0(q): return pltpu.make_async_copy(x_hbm.at[0, :, pl.ds(q * c0, c0)], xbuf.at[0, :, pl.ds(q * c0, c0)], psem.at[3 + q])
        def wr(s0, n, j):
            idx = (pl.ds(2 * s0, 2 * n), pl.ds(j * wr_rows, wr_rows))
            return pltpu.make_async_copy(obuf.at[idx], o_hbm.at[idx], wsem.at[0])
        def wrf(i, c0, nc):
            idx = (2 * (NS - 1) + i, slice(None), pl.ds(c0, nc))
            return pltpu.make_async_copy(obuf.at[idx], o_hbm.at[idx], wsem.at[0])
        pc = [pltpu.make_async_copy(w_hbm, w_ref, psem.at[0]), pltpu.make_async_copy(g_hbm, g_ref, psem.at[1]), pltpu.make_async_copy(b_hbm, b_ref, psem.at[2])]
        for c in pc: c.start()
        if dma:
            for q in range(split0): rd0(q).start()
            for s in range(1, NS): rd(s).start()
        for c in pc: c.wait()
        g = g_ref[...].astype(f32).reshape(1, D); b = b_ref[...].astype(f32).reshape(1, D)
        wt = w_ref[...].astype(f32).T
        bias_ref[...] = jnp.broadcast_to(jnp.sum(wt * b, axis=1, keepdims=True), bias_ref.shape)
        wg = wt * g
        t = [wg[:, k * 128:(k + 1) * 128] for k in range(4)]
        t3q = jnp.concatenate([wg[:, 384:448], wg[:, 512:]], axis=1)
        ar[...] = pk(wg[:, 448:])
        for m in range(1, 8):
            L = [acomb(m, a1[:H], a2_[:H], a1[H:], a2_[H:]) for a1, a2_ in [(t[0], t[2]), (t[1], t[3]), (t[1], t3q)]]
            nv = 1 if m in (3, 6) else 2
            if m in two:
                for v in range(nv):
                    for n in range(1, 8):
                        if v == 1 and n in (3, 6): continue
                        a2[two.index(m), v, n - 1] = pk(acomb(n, L[0][:H // 2], L[1 + v][:H // 2], L[0][H // 2:], L[1 + v][H // 2:]))
            else:
                for j in range(1 + nv): at[m - 1, j] = pk(L[j])

        def ldx(s, p, r0=0, r1=D): return xbuf[s, r0:r1, p * 256:(p + 1) * 256].astype(f32)
        def stats(s, p):
            x = ldx(s, p)
            c = x[0:1]
            xc = x - c
            d = jnp.sum(xc, axis=0, keepdims=True) * (1.0 / D)
            var = jnp.sum(xc * xc, axis=0, keepdims=True) * (1.0 / D) - d * d
            return c + d, lax.rsqrt(jnp.maximum(var, 0.0) + EPS)
        def norm(s, p, st, r0, r1): return (ldx(s, p, r0, r1) - st[0]) * st[1]
        def half(s, p, st, k):
            if k == 0: return norm(s, p, st, 0, 256)
            y = norm(s, p, st, 256, 576)
            tail = jnp.concatenate([y[192:256, :128] - y[192:256, 128:], y[256:, 128:] - y[256:, :128]], axis=1)
            return jnp.concatenate([y[:192], tail], axis=0)
        def prod(m, rhs):
            rp = rhs[:, :128].astype(bf16); rq = rhs[:, 128:].astype(bf16)
            a0 = up(at[m - 1, 0])
            mp = jnp.dot(jnp.concatenate([a0, up(at[m - 1, 1])], axis=1), rp, preferred_element_type=f32)
            mq = jnp.dot(jnp.concatenate([a0, up(at[m - 1, 1 if m in (3, 6) else 2])], axis=1), rq, preferred_element_type=f32)
            return jnp.concatenate([mp, mq], axis=1)
        def slice_(s, st, sns, maybe_last, hook, wstep, d0):
            nk = 4 * nch * len(sns)
            deps = [d0 + i * (d1 - d0) / nk for i in range(nk)]
            rr = []; nst = [None] * (4 * len(sns))
            never = jnp.broadcast_to(st[0][1], (8, 256)) < 0.0
            rows = D // nch
            sacc = {}
            def stat_chunk(k, dep):
                p, j = divmod(k, nch)
                x = ldx(sns[p // 4], p % 4, j * rows, (j + 1) * rows)
                if j == 0:
                    sacc[p] = [jnp.broadcast_to(x[0:1], (8, 256)), None, None]
                c, s1, s2 = sacc[p]
                c = jnp.where(never, dep, c)
                for r in range(0, rows, 8):
                    xc = x[r:r + 8] - c
                    s1 = xc if s1 is None else s1 + xc
                    s2 = xc * xc if s2 is None else s2 + xc * xc
                sacc[p] = [sacc[p][0], s1, s2]
                if j == nch - 1:
                    d = jnp.sum(s1, axis=0, keepdims=True) * (1.0 / D)
                    var = jnp.sum(s2, axis=0, keepdims=True) * (1.0 / D) - d * d
                    nst[p] = (sacc[p][0][0:1] + d, lax.rsqrt(jnp.maximum(var, 0.0) + EPS))
            clock = [1.0]; nxt = [0]; marks = []; hooked = [wstep == 0]
            def tick(val, dur):
                marks.append((clock[0], dur, val)); clock[0] += dur
                if not hooked[0] and clock[0] > wstep:
                    hook(); hooked[0] = True
                while hooked[0] and nxt[0] < nk and deps[nxt[0]] < clock[0] - 1e-9:
                    d = deps[nxt[0]]
                    t0, du, v = [mk for mk in marks if mk[0] <= d + 1e-9][-1]
                    r0 = min(int((d - t0) / du * v.shape[0]) // 8 * 8, v.shape[0] - 8)
                    stat_chunk(nxt[0], v[r0:r0 + 8]); nxt[0] += 1
            Bc = {}
            def Bq(q):
                def Bm(k, j):
                    if (q, k, j) not in Bc: Bc[q, k, j] = half(s, 2 * q + j, st[2 * q + j], k)
                    return Bc[q, k, j]
                return Bm
            M = [{}, {}]
            todo = [dict(OUTS), dict(OUTS)]
            for tok in steps:
                if tok == "r":
                    for p in range(4):
                        y = norm(s, p, st[p], 448, 576)
                        rt = jnp.concatenate([y[:64, 128:], y[64:, :128]], axis=0).astype(bf16)
                        rr.append(jnp.dot(up(ar[...]), rt, preferred_element_type=f32) + bias_ref[...])
                    for q in range(2): M[q]["r"] = None
                elif tok[-1] == "x":
                    m = int(tok[0]); ti = two.index(m)
                    U = [bcomb(m, Bq(q)) for q in range(2)]
                    N = {}
                    for ch in o2:
                        n = int(ch)
                        rhs = bcomb(n, lambda k, j: U[j][k * 128:(k + 1) * 128])
                        vq = 0 if (m in (3, 6) or n in (3, 6)) else 1
                        N[n] = jnp.concatenate([jnp.dot(up(a2[ti, 0, n - 1]), rhs[:, :128].astype(bf16), preferred_element_type=f32),
                                                jnp.dot(up(a2[ti, vq, n - 1]), rhs[:, 128:].astype(bf16), preferred_element_type=f32)], axis=1)
                        tick(N[n], 0.25)
                    for q in range(2):
                        M[q][m] = jnp.concatenate([chain([(OUTS[i, q][n], N[n]) for n in N if n in OUTS[i, q]]) for i in range(2)], axis=0)
                else:
                    m = int(tok[0]); q = "ab".index(tok[1])
                    M[q][m] = prod(m, bcomb(m, Bq(q)))
                    tick(M[q][m], 1.0)
                for q in range(2):
                    for key in list(todo[q]):
                        if "r" in M[q] and all(n in M[q] for n in OUTS[key]):
                            i, j = key; p = 2 * q + j
                            r = rr[p][i * H:(i + 1) * H]
                            val = chain([(1, jnp.concatenate([r, r], axis=1)) if n == "r" else (OUTS[key][n], M[q][n]) for n in M[q] if n == "r" or n in OUTS[key]])
                            obuf[2 * s + i, :, p * 256:(p + 1) * 256] = val.astype(bf16)
                            del todo[q][key]
                            if dma and maybe_last and fine:
                                @pl.when(s == NS - 1)
                                def _(): wrf(i, p * 256, 256).start()
            assert nxt[0] == nk and not todo[0] and not todo[1], (nxt, clock)
            return [nst[4 * i:4 * i + 4] for i in range(len(sns))]

        st = [None] * 4
        for p in range(4):
            if dma and (p * 256) % c0 == 0: rd0(p * 256 // c0).wait()
            st[p] = stats(0, p)
        have = [st]; nxt_s = 1
        for s in range(peel):
            upto = 1 + ((peel + unroll - 1) * (s + 1)) // peel
            sns = list(range(nxt_s, upto)); nxt_s = upto
            def hk(sns=sns):
                if dma:
                    for k in sns: rd(k).wait()
            if s > 0: hk()
            have = have[1:] + slice_(s, have[0], sns, False, hk, pwstep if s == 0 else 0, pd0 if s == 0 else d0)
        if peel == 0:
            for u in range(1, unroll):
                if dma: rd(u).wait()
                have.append([stats(u, p) for p in range(4)])
        nit = (NS - peel) // unroll
        assert nit * unroll + peel == NS and len(have) == unroll
        def body(i, st):
            s0 = peel + i * unroll
            def wait(u):
                if not dma: return
                @pl.when(i < nit - 1)
                def _(): rd(s0 + unroll + u).wait()
            if wstep == 0:
                for u in range(unroll): wait(u)
            sn0 = jnp.minimum(s0 + unroll, NS - unroll)
            out = []
            for u in range(unroll):
                s = s0 + u
                if dma:
                    for n in sorted(set(b - a for a, b in groups)):
                        ends = [b for a, b in groups if b - a == n and (b - peel) % unroll == u and b < NS]
                        if not ends: continue
                        cond = functools.reduce(jnp.logical_or, [s == e for e in ends])
                        @pl.when(cond)
                        def _():
                            for j in range(wn): wr(s - n, n, j).start()
                out += slice_(s, st[u], [sn0 + u], u == unroll - 1, functools.partial(wait, u), wstep, d0)
            return out
        lax.fori_loop(0, nit, body, have)
        if dma:
            for a, b in groups:
                if b == NS:
                    for j in range(wn): wr(a, b - a, j).start()
            pltpu.make_async_copy(obuf, o_hbm, wsem.at[0]).wait()
        else:
            wr(0, 1, 0).start(); wr(0, 1, 0).wait()

    def f(x, g, b, w):
        xt = jnp.transpose(x, (1, 2, 0))
        anys = pl.BlockSpec(memory_space=pl.ANY)
        o = pl.pallas_call(kern,
            in_specs=[anys, anys, anys, anys],
            out_specs=anys,
            out_shape=jax.ShapeDtypeStruct((2 * NS, H, 1024), xt.dtype),
            scratch_shapes=[pltpu.VMEM(xt.shape, bf16), pltpu.VMEM((2 * NS, H, 1024), bf16),
                            pltpu.VMEM((D,), bf16), pltpu.VMEM((D,), bf16), pltpu.VMEM((D, D), bf16),
                            pltpu.VMEM((7, 3, H // 2, 128), u32), pltpu.VMEM((max(1, len(two)), 2, 7, H // 4, 128), u32),
                            pltpu.VMEM((D // 2, 128), u32), pltpu.VMEM((D, 128), f32),
                            pltpu.SemaphoreType.DMA((NS,)), pltpu.SemaphoreType.DMA((7,)), pltpu.SemaphoreType.DMA((1,))],
            compiler_params=pltpu.CompilerParams(vmem_limit_bytes=100 * 2**20, flags=flags, disable_bounds_checks=nobc),
        )(xt, g, b, w)
        return jnp.transpose(o.reshape(NS, D, 1024), (2, 0, 1))
    return f
FL = {'XLA_TPU_RESCHEDULE_DMA_DONES': True}


_impl = make(sched='2x 5x 1a 3a r 6a 4a 7a 1b 3b 6b 4b 7b', d0=4.5, d1=14, nch=24, unroll=2, peel=4, pd0=4.5,
             groups=(15, 22, 26, 28, 29, 30, 31))


@jax.jit
def pallas_standalone__layernorm_linear__sampling_kernel(x, g, b, w):
    return _impl(x, g, b, w)
```

```python
import functools

import jax
import jax.numpy as jnp
from jax import lax
import jax.experimental.pallas as pl
import jax.experimental.pallas.tpu as pltpu

NS, D, NT = 32, 576, 1024
H = D // 2
PW = 256
NPAIR = NT // PW
EPS = 1e-5
F32, BF16, U32 = jnp.float32, jnp.bfloat16, jnp.uint32

STEPS = "2x 5x 1x 3a r 6a 4a 7a 3b 6b 4b 7b".split()
LEVEL2_ORDER = (2, 1, 5, 3, 6, 4, 7)
LEVEL2 = sorted(int(t[0]) for t in STEPS if t.endswith("x"))
COMBINE = {
    (0, 1): {3: 1, 5: 1},
    (1, 0): {2: 1, 4: 1},
    (0, 0): {1: 1, 4: 1, 5: -1, 7: 1},
    (1, 1): {1: 1, 2: -1, 3: 1, 6: 1},
}
FIRST_K_HALF_ONLY = (3, 6)

UNROLL = 3
PEEL_STATS = (1, 1, 2, 1, 2)
STAT_ROWS = 24
STAT_BEGIN, STAT_END = 5.0, 12.7
FIRST_WAIT, FIRST_STAT_BEGIN = 6.0, 5.25
W_BLOCKS = ((0, 128), (256, 384), (128, 256), (384, 576))
X0_BLOCKS = 4
WRITES = (
    (15, 0, 3, 8), (16, 3, 3, 8), (18, 6, 3, 8), (19, 9, 3, 8), (21, 12, 3, 8), (22, 15, 3, 8),
    (24, 18, 3, 8), (25, 21, 3, 8), (27, 24, 3, 8), (29, 27, 2, 8), (30, 29, 1, 24), (31, 30, 1, 24),
)
COPIES_PER_STEP = 12


def _a1_keys():
    return [(m, t) for t in range(3) for m in range(1, 8)
            if m not in LEVEL2 and not (t == 2 and m in FIRST_K_HALF_ONLY)]


def _a2_keys():
    return [(m, v, n) for m in LEVEL2 for v in range(2) for n in range(1, 8)
            if not (v == 1 and (m in FIRST_K_HALF_ONLY or n in FIRST_K_HALF_ONLY))]


def _left(m, k0, k1):
    h = k0.shape[0] // 2
    a11, a12, a21, a22 = k0[:h], k1[:h], k0[h:], k1[h:]
    return {
        1: lambda: a11 + a22, 2: lambda: a21 + a22, 3: lambda: a11, 4: lambda: a22,
        5: lambda: a11 + a12, 6: lambda: a21 - a11, 7: lambda: a12 - a22,
    }[m]()


def _right(m, blk):
    return {
        1: lambda: blk(0, 0) + blk(1, 1), 2: lambda: blk(0, 0),
        3: lambda: blk(0, 1) - blk(1, 1), 4: lambda: blk(1, 0) - blk(0, 0),
        5: lambda: blk(1, 1), 6: lambda: blk(0, 0) + blk(0, 1),
        7: lambda: blk(1, 0) + blk(1, 1),
    }[m]()


def _signed_sum(terms):
    sign, acc = terms[0]
    for s, v in terms[1:]:
        if sign > 0:
            acc = acc + v if s > 0 else acc - v
        elif s > 0:
            acc, sign = v - acc, 1
        else:
            acc = acc + v
    assert sign > 0
    return acc


def _pack(v):
    return pltpu.bitcast(v.astype(BF16), U32)


def _unpack(v):
    return pltpu.bitcast(v, BF16)


def _dot(a, y):
    return jnp.dot(a, y, preferred_element_type=F32)


def _stat_add(x, shift, s1, s2):
    for r in range(0, x.shape[0], 8):
        xc = x[r:r + 8] - shift
        s1 = xc if s1 is None else s1 + xc
        s2 = xc * xc if s2 is None else s2 + xc * xc
    return s1, s2


def _stat_finish(shift, s1, s2):
    d = jnp.sum(s1, axis=0, keepdims=True) * (1.0 / D)
    var = jnp.sum(s2, axis=0, keepdims=True) * (1.0 / D) - d * d
    return shift[0:1] + d, lax.rsqrt(jnp.maximum(var, 0.0) + EPS)


def _stats_to_rows(stats):
    row = lax.broadcasted_iota(jnp.int32, (8, PW), 0)
    v = jnp.broadcast_to(stats[0][0], (8, PW))
    for k in range(1, 8):
        v = jnp.where(row == k, stats[k // 2][k % 2], v)
    return v


def _rows_to_stats(v):
    return [(v[2 * p:2 * p + 1], v[2 * p + 1:2 * p + 2]) for p in range(NPAIR)]


def _kernel(x_hbm, g_hbm, b_hbm, w_hbm, o_hbm,
            xbuf, obuf, g_ref, b_ref, w_ref, a1_ref, a2_ref, ar_ref, bias_ref,
            x_sems, first_sems, o_sem):
    a1_keys, a2_keys = _a1_keys(), _a2_keys()

    def read(s):
        return pltpu.make_async_copy(x_hbm.at[s], xbuf.at[s], x_sems.at[s - 1])

    def write(*idx):
        return pltpu.make_async_copy(obuf.at[idx], o_hbm.at[idx], o_sem.at[0])

    def load(s, p, r0, r1):
        return xbuf[s, r0:r1, p * PW:(p + 1) * PW].astype(F32)

    x0_rows = D // X0_BLOCKS
    first = [(g_hbm, g_ref), (b_hbm, b_ref)]
    first += [(w_hbm.at[pl.ds(k0, k1 - k0)], w_ref.at[pl.ds(k0, k1 - k0)]) for k0, k1 in W_BLOCKS]
    first += [(x_hbm.at[0, pl.ds(q * x0_rows, x0_rows)], xbuf.at[0, pl.ds(q * x0_rows, x0_rows)])
              for q in range(X0_BLOCKS)]
    first = [pltpu.make_async_copy(src, dst, first_sems.at[i]) for i, (src, dst) in enumerate(first)]
    for copy in first:
        copy.start()
    for s in range(1, NS):
        read(s).start()

    first[0].wait()
    first[1].wait()
    g = g_ref[...].astype(F32).reshape(1, D)
    b = b_ref[...].astype(F32).reshape(1, D)
    tile = {}

    def k_halves(t):
        lo, hi = ((0, 2), (1, 3), (1, 4))[t]
        return tile[lo], tile[hi]

    def store_level1(t):
        for i, (m, mt) in enumerate(a1_keys):
            if mt == t:
                a1_ref[i] = _pack(_left(m, *k_halves(t)))

    bias = 0.0
    for n, (k0, k1) in enumerate(W_BLOCKS):
        first[2 + n].wait()
        wt = w_ref[k0:k1].astype(F32).T
        wb = wt * b[:, k0:k1]
        wg = wt * g[:, k0:k1]
        tile[k0 // 128] = wg[:, :128]
        bias = bias + wb[:, :128]
        if k1 == D:
            tile[4] = jnp.concatenate([wg[:, 384 - k0:448 - k0], wg[:, 512 - k0:]], axis=1)
            ar_ref[...] = _pack(wg[:, 448 - k0:])
            bias = (jnp.sum(bias, axis=1, keepdims=True)
                    + jnp.sum(wb[:, 512 - k0:], axis=1, keepdims=True))
            bias_ref[...] = jnp.broadcast_to(bias, bias_ref.shape)
        if n == 1:
            store_level1(0)
    store_level1(1)
    store_level1(2)
    for m in LEVEL2:
        left = [_left(m, *k_halves(t)) for t in range(3)]
        for i, (km, v, n) in enumerate(a2_keys):
            if km == m:
                a2_ref[i] = _pack(_left(n, left[0], left[1 + v]))

    def a1(m, t):
        return _unpack(a1_ref[a1_keys.index((m, t) if (m, t) in a1_keys else (m, 1))])

    def a2(m, v, n):
        return _unpack(a2_ref[a2_keys.index((m, v, n) if (m, v, n) in a2_keys else (m, 0, n))])

    def do_slice(s, stats, later, *, stat_begin=STAT_BEGIN, wait_later=None,
                 start_writes=None, may_be_last=False):
        per_pair = D // STAT_ROWS
        n_chunks = len(later) * NPAIR * per_pair
        new_stats, sums = [], {}
        never = jnp.broadcast_to(stats[0][1], (8, PW)) < 0.0
        issued = []
        state = {"round": 0.0, "chunk": 0, "wait": wait_later}

        def stat_chunk(k, anchor):
            p, j = divmod(k, per_pair)
            x = load(later[p // NPAIR], p % NPAIR, j * STAT_ROWS, (j + 1) * STAT_ROWS)
            if j == 0:
                sums[p] = (jnp.broadcast_to(x[0:1], (8, PW)), None, None)
            shift, s1, s2 = sums[p]
            sums[p] = (shift, *_stat_add(x, jnp.where(never, anchor, shift), s1, s2))
            if j == per_pair - 1:
                new_stats.append(_stat_finish(*sums[p]))

        def advance(result, rounds):
            issued.append((state["round"], rounds, result))
            state["round"] += rounds
            if state["wait"] is not None and state["round"] > FIRST_WAIT:
                state["wait"]()
                state["wait"] = None
            while state["wait"] is None and state["chunk"] < n_chunks:
                when = stat_begin + state["chunk"] * (STAT_END - stat_begin) / n_chunks
                if when >= state["round"] - 1e-9:
                    break
                t0, dt, v = [e for e in issued if e[0] <= when + 1e-9][-1]
                r = min(int((when - t0) / dt * v.shape[0]) // 8 * 8, v.shape[0] - 8)
                stat_chunk(state["chunk"], v[r:r + 8])
                state["chunk"] += 1

        def normed(p, r0, r1):
            return (load(s, p, r0, r1) - stats[p][0]) * stats[p][1]

        blocks = {}

        def block(quad, k, j):
            p = 2 * quad + j
            if (p, k) not in blocks:
                if k == 0:
                    blocks[p, k] = normed(p, 0, 256)
                else:
                    y = normed(p, 256, D)
                    tail = jnp.concatenate([y[192:256, :128] - y[192:256, 128:],
                                            y[256:, 128:] - y[256:, :128]], axis=1)
                    blocks[p, k] = jnp.concatenate([y[:192], tail], axis=0)
            return blocks[p, k]

        products = [{}, {}]
        pending = [list(COMBINE), list(COMBINE)]
        shared = []
        for n_step, step in enumerate(STEPS):
            if start_writes is not None:
                start_writes(n_step)
            if step == "r":
                for p in range(NPAIR):
                    y = normed(p, 448, D)
                    y = jnp.concatenate([y[:64, 128:], y[64:, :128]], axis=0).astype(BF16)
                    shared.append(_dot(_unpack(ar_ref[...]), y) + bias_ref[...])
                for quad in range(2):
                    products[quad]["r"] = None
            elif step.endswith("x"):
                m = int(step[0])
                right = [_right(m, functools.partial(block, quad)) for quad in range(2)]
                sub = {}
                for n in LEVEL2_ORDER:
                    y = _right(n, lambda k, j: right[j][k * 128:(k + 1) * 128])
                    sub[n] = jnp.concatenate([_dot(a2(m, 0, n), y[:, :128].astype(BF16)),
                                              _dot(a2(m, 1, n), y[:, 128:].astype(BF16))], axis=1)
                    advance(sub[n], 0.25)
                for quad in range(2):
                    products[quad][m] = jnp.concatenate(
                        [_signed_sum([(COMBINE[i, quad][n], v) for n, v in sub.items()
                                      if n in COMBINE[i, quad]]) for i in range(2)], axis=0)
            else:
                m, quad = int(step[0]), "ab".index(step[1])
                y = _right(m, functools.partial(block, quad))
                yp, yq = y[:, :128].astype(BF16), y[:, 128:].astype(BF16)
                a = a1(m, 0)
                products[quad][m] = jnp.concatenate(
                    [_dot(jnp.concatenate([a, a1(m, 1)], axis=1), yp),
                     _dot(jnp.concatenate([a, a1(m, 2)], axis=1), yq)], axis=1)
                advance(products[quad][m], 1.0)

            for quad in range(2):
                have = products[quad]
                for i, j in list(pending[quad]):
                    signs = COMBINE[i, j]
                    if "r" not in have or any(m not in have for m in signs):
                        continue
                    pending[quad].remove((i, j))
                    p = 2 * quad + j
                    r = shared[p][i * H:(i + 1) * H]
                    out = _signed_sum([
                        (1, jnp.concatenate([r, r], axis=1)) if m == "r" else (signs[m], v)
                        for m, v in have.items() if m == "r" or m in signs])
                    obuf[2 * s + i, :, p * PW:(p + 1) * PW] = out.astype(BF16)
                    if may_be_last:
                        @pl.when(s == NS - 1)
                        def _():
                            write(2 * (NS - 1) + i, slice(None), pl.ds(p * PW, PW)).start()

        assert state["chunk"] == n_chunks and not pending[0] and not pending[1]
        return [new_stats[NPAIR * i:NPAIR * (i + 1)] for i in range(len(later))]

    sums = {}
    for q in range(X0_BLOCKS):
        first[2 + len(W_BLOCKS) + q].wait()
        for p in range(NPAIR):
            x = load(0, p, q * x0_rows, (q + 1) * x0_rows)
            if q == 0:
                sums[p] = (jnp.broadcast_to(x[0:1], (8, PW)), None, None)
            sums[p] = (sums[p][0], *_stat_add(x, *sums[p]))
    ready = [[_stat_finish(*sums[p]) for p in range(NPAIR)]]

    peel = len(PEEL_STATS)
    for s, n in enumerate(PEEL_STATS):
        later = list(range(s + len(ready), s + len(ready) + n))

        def wait_later(later=later):
            for k in later:
                read(k).wait()

        if s == 0:
            new = do_slice(s, ready[0], later, stat_begin=FIRST_STAT_BEGIN, wait_later=wait_later)
        else:
            wait_later()
            new = do_slice(s, ready[0], later)
        ready = ready[1:] + new

    n_iter = (NS - peel) // UNROLL
    assert peel + n_iter * UNROLL == NS and len(ready) == UNROLL

    def start_writes(s, u, n_step):
        due = [e for e in WRITES
               if (e[0] - peel) % UNROLL == u and n_step * COPIES_PER_STEP * e[3] < H]
        for n, rows in sorted({e[2:] for e in due}):
            group = [e for e in due if e[2:] == (n, rows)]
            issue = functools.reduce(jnp.logical_or, [s == e[0] for e in group])
            s0 = group[0][1]
            for e in group[1:]:
                s0 = jnp.where(s == e[0], e[1], s0)

            @pl.when(issue)
            def _():
                for j in range(n_step * COPIES_PER_STEP, (n_step + 1) * COPIES_PER_STEP):
                    write(pl.ds(2 * s0, 2 * n), pl.ds(j * rows, rows)).start()

    def body(it, carry):
        stats = [_rows_to_stats(v) for v in carry]
        s0 = peel + it * UNROLL
        for u in range(UNROLL):
            @pl.when(it < n_iter - 1)
            def _():
                read(s0 + UNROLL + u).wait()
        later0 = jnp.minimum(s0 + UNROLL, NS - UNROLL)
        new = []
        for u in range(UNROLL):
            s = s0 + u
            new += do_slice(s, stats[u], [later0 + u],
                            start_writes=functools.partial(start_writes, s, u),
                            may_be_last=u == UNROLL - 1)
        return [_stats_to_rows(v) for v in new]

    lax.fori_loop(0, n_iter, body, [_stats_to_rows(v) for v in ready])

    pltpu.make_async_copy(obuf, o_hbm, o_sem.at[0]).wait()


@jax.jit
def pallas_standalone__layernorm_linear__sampling_kernel(
    x: jax.Array,
    g: jax.Array,
    b: jax.Array,
    w: jax.Array,
):
    assert x.shape == (NT, NS, D) and g.shape == b.shape == (D,) and w.shape == (D, D)
    assert x.dtype == g.dtype == b.dtype == w.dtype == BF16
    in_hbm = pl.BlockSpec(memory_space=pl.ANY)
    out = pl.pallas_call(
        _kernel,
        in_specs=[in_hbm] * 4,
        out_specs=in_hbm,
        out_shape=jax.ShapeDtypeStruct((2 * NS, H, NT), BF16),
        scratch_shapes=[
            pltpu.VMEM((NS, D, NT), BF16),
            pltpu.VMEM((2 * NS, H, NT), BF16),
            pltpu.VMEM((D,), BF16),
            pltpu.VMEM((D,), BF16),
            pltpu.VMEM((D, D), BF16),
            pltpu.VMEM((len(_a1_keys()), H // 2, 128), U32),
            pltpu.VMEM((len(_a2_keys()), H // 4, 128), U32),
            pltpu.VMEM((D // 2, 128), U32),
            pltpu.VMEM((D, 128), F32),
            pltpu.SemaphoreType.DMA((NS - 1,)),
            pltpu.SemaphoreType.DMA((2 + len(W_BLOCKS) + X0_BLOCKS,)),
            pltpu.SemaphoreType.DMA((1,)),
        ],
        compiler_params=pltpu.CompilerParams(vmem_limit_bytes=100 * 2**20),
    )(jnp.transpose(x, (1, 2, 0)), g, b, w)
    return jnp.transpose(out.reshape(NS, D, NT), (2, 0, 1))
```
